```python
import jax
import jax.numpy as jnp

def _softmax(x, axis=-1):
    return jax.nn.softmax(x, axis=axis)
def _gelu(x):
    return jax.nn.gelu(x, approximate=True)
def _silu(x):
    return jax.nn.silu(x)
def _sigmoid(x):
    return jax.nn.sigmoid(x)
def _layernorm(x, axis=-1, eps=1e-5):
    m = jnp.mean(x, axis=axis, keepdims=True)
    v = jnp.var(x, axis=axis, keepdims=True)
    return (x - m) / jnp.sqrt(v + eps)
def _scatter_add(tgt, idx, src, axis=0):
    return tgt.at[idx].add(src)
def _segment_sum(src, seg, n):
    return jax.ops.segment_sum(src, seg, n)
class _Rng:
    def __init__(self, key):
        self._k = key
    def _next(self):
        self._k, sub = jax.random.split(self._k)
        return sub
    def normal(self, shape):
        return jax.random.normal(self._next(), shape, dtype=jnp.bfloat16)
    def randint(self, lo, hi, shape):
        return jax.random.randint(self._next(), shape, lo, hi, dtype=jnp.int32)
    def uniform(self, shape, lo=0.0, hi=1.0):
        return jax.random.uniform(self._next(), shape, jnp.bfloat16, lo, hi)
    def permutation(self, n):
        return jax.random.permutation(self._next(), n)


kernel_name = 'recurrent_scan__sliding_block_cached__glu_gated_glu__decode'

def setup_inputs():
    _rng = _Rng(jax.random.key(int.from_bytes(__import__("os").urandom(4), "little")))
    _w = (lambda a: (lambda t: t.astype(jnp.bfloat16) if jnp.issubdtype(t.dtype, jnp.floating) else t)(jnp.asarray(a)))
    def _A_setup():
        B, Sq, D = 1, 1, 576
        Hq, Hkv, Sk, Dh = 32, 16, 65536, 128
        assert Hq % Hkv == 0, (Hq, Hkv)
        return {
            "x": _w((lambda *s: _rng.normal(s) * 0.05)(B, Sq, D)),
            "k_cache": _w((lambda *s: _rng.normal(s) * 0.05)(B, Hkv, Sk, Dh)),
            "v_cache": _w((lambda *s: _rng.normal(s) * 0.05)(B, Hkv, Sk, Dh)),
            "wq": _w((lambda *s: _rng.normal(s) * 0.05)(D, Hq * Dh) * (D ** -0.5)),
            "wo": _w((lambda *s: _rng.normal(s) * 0.05)(Hq * Dh, D) * ((Hq * Dh) ** -0.5)),
        }
    _A_in = _A_setup()

    def _B_setup():
        B, S, D, F = 1, 1, 576, 4608
        return {
            "x": _w((lambda *s: _rng.normal(s) * 0.05)(B, S, D)),
            "w_gate": _w((lambda *s: _rng.normal(s) * 0.05)(D, F)),
            "w_up": _w((lambda *s: _rng.normal(s) * 0.05)(D, F)),
            "w_down": _w((lambda *s: _rng.normal(s) * 0.05)(F, D)),
        }
    _B_in = _B_setup()

    return {
        "A_x": _A_in["x"],
        "A_k_cache": _A_in["k_cache"],
        "A_v_cache": _A_in["v_cache"],
        "A_wq": _A_in["wq"],
        "A_wo": _A_in["wo"],
        "B_x": _B_in["x"],
        "B_w_gate": _B_in["w_gate"],
        "B_w_up": _B_in["w_up"],
        "B_w_down": _B_in["w_down"],
    }

def reference(A_x, A_k_cache, A_v_cache, A_wq, A_wo, B_x, B_w_gate, B_w_up, B_w_down):
    def _A_ref(x, k_cache, v_cache, wq, wo):
        B, Sq, D = x.shape
        Hq, Dh = 32, 128
        Hkv, Sk = k_cache.shape[1], k_cache.shape[2]
        W = min(4096, max(256, Sk // 4))
        rep = Hq // Hkv
        q = (lambda x, *d: x.transpose(*d))((x @ wq).reshape(B, Sq, Hq, Dh), 0, 2, 1, 3)
        k = jnp.repeat(k_cache[:, :, Sk - W:, :], rep, axis=1)
        v = jnp.repeat(v_cache[:, :, Sk - W:, :], rep, axis=1)
        scores = jnp.einsum("bhqd,bhkd->bhqk", q, k) * (Dh ** -0.5)
        p = _softmax(scores, axis=-1)
        o = jnp.einsum("bhqk,bhkd->bhqd", p, v)
        return (lambda x, *d: x.transpose(*d))(o, 0, 2, 1, 3).reshape(B, Sq, Hq * Dh) @ wo

    def _B_ref(x, w_gate, w_up, w_down):
        g = jnp.einsum("bsd,df->bsf", x, w_gate)
        u = jnp.einsum("bsd,df->bsf", x, w_up)
        h = _sigmoid(g) * u
        return jnp.einsum("bsf,fd->bsd", h, w_down)

    x = A_x
    xn = _layernorm(x, axis=-1)
    s = _A_ref(xn, A_k_cache, A_v_cache, A_wq, A_wo)
    g = _silu(_B_ref(xn, B_w_gate, B_w_up, B_w_down))
    return x + s * g
```

```python
import functools

import jax
import jax.numpy as jnp
from jax import lax
import jax.experimental.pallas as pl
import jax.experimental.pallas.tpu as pltpu

_BF = jnp.bfloat16
_F32 = jnp.float32
_NT = (((1,), (1,)), ((), ()))
_NN = (((1,), (0,)), ((), ()))

_HQ, _DH = 32, 128
_STEP = 512
_WO_SLABS = (15, 10, 4, 2, 1)


def _kernel(x_hbm, k_hbm, v_hbm, wq_hbm, woT_hbm, wg_hbm, wu_hbm, wdT_hbm, o_ref,
            xb, kb, vb, wq, wo, wg, wu, wd, q_s, p_s, l_s, g_s, h_s, o_s, sems, osem,
            *, bounds):
    D = xb.shape[1]
    HKV, W, DH = kb.shape
    SK = k_hbm.shape[2]
    F = wg.shape[1]
    GRP = 2 * DH
    nwo = len(bounds) - 1

    def cp(src, dst, i):
        return pltpu.make_async_copy(src, dst, sems.at[i])

    def cwo(i):
        a, b = bounds[i], bounds[i + 1]
        return pltpu.make_async_copy(
            woT_hbm.at[:, pl.ds(a, b - a)], wo.at[:, pl.ds(a, b - a)], osem.at[i])

    mk = dict(
        x=lambda: cp(x_hbm, xb, 0),
        wq=lambda: cp(wq_hbm, wq, 1),
        k=lambda: cp(k_hbm.at[0, :, pl.ds(SK - W, W), :], kb, 2),
        v=lambda: cp(v_hbm.at[0, :, pl.ds(SK - W, W), :], vb, 3),
        wg=lambda: cp(wg_hbm, wg, 4),
        wu=lambda: cp(wu_hbm, wu, 5),
        wd=lambda: cp(wdT_hbm, wd, 6),
    )
    for i in range(nwo):
        mk[f"wo{i}"] = functools.partial(cwo, i)
    todo = ["x", "wq", "k", "v", "wg", "wu", "wd"] + [f"wo{i}" for i in range(nwo)]

    def start(n=1):
        for _ in range(n):
            if todo:
                mk[todo.pop(0)]().start()

    def wait(name):
        mk[name]().wait()

    start(3)
    wait("x")
    x = xb[...].astype(_F32)
    m = jnp.mean(x, axis=-1, keepdims=True)
    xc = x - m
    var = jnp.mean(xc * xc, axis=-1, keepdims=True)
    xn = xc / jnp.sqrt(var + 1e-5)
    xn8 = jnp.broadcast_to(xn, (8, D)).astype(_BF)
    row = lax.broadcasted_iota(jnp.int32, (8, DH), 0)

    wait("wq")

    def qbody(h, c):
        off = pl.multiple_of(h * GRP, GRP)
        q = lax.dot_general(xn8, wq[:, pl.ds(off, GRP)], _NN, preferred_element_type=_F32)
        q_s[h] = jnp.where(row == 0, q[:, :DH], q[:, DH:])
        return c

    lax.fori_loop(0, HKV, qbody, 0)
    start()
    wait("k")

    def sbody(h, c):
        q = q_s[h].astype(_BF)
        s = lax.dot_general(q, kb[h], _NT, preferred_element_type=_F32) * (DH ** -0.5)
        mx = jnp.max(s, axis=-1, keepdims=True)
        p = jnp.exp(s - mx)
        l_s[h] = jnp.broadcast_to(jnp.sum(p, axis=-1, keepdims=True), (8, DH))
        p_s[h] = p
        return c

    lax.fori_loop(0, HKV, sbody, 0)
    start()
    wait("v")
    start()

    def pvbody(h, c):
        o = lax.dot_general(p_s[h].astype(_BF), vb[h], _NN, preferred_element_type=_F32) / l_s[h]
        off = pl.multiple_of(h * GRP, GRP)
        o_s[:, pl.ds(off, GRP)] = jnp.concatenate(
            [jnp.broadcast_to(o[0:1], (8, DH)), jnp.broadcast_to(o[1:2], (8, DH))], axis=1)
        return c

    lax.fori_loop(0, HKV, pvbody, 0)
    start()
    wait("wg")

    def gbody(j, c):
        off = pl.multiple_of(j * _STEP, _STEP)
        g = lax.dot_general(xn8, wg[:, pl.ds(off, _STEP)], _NN, preferred_element_type=_F32)
        g_s[:, pl.ds(off, _STEP)] = jax.nn.sigmoid(g)
        return c

    lax.fori_loop(0, F // _STEP, gbody, 0)
    start()
    wait("wu")
    start()

    def ubody(j, c):
        off = pl.multiple_of(j * _STEP, _STEP)
        u = lax.dot_general(xn8, wu[:, pl.ds(off, _STEP)], _NN, preferred_element_type=_F32)
        h_s[:, pl.ds(off, _STEP)] = g_s[:, pl.ds(off, _STEP)] * u
        return c

    lax.fori_loop(0, F // _STEP, ubody, 0)
    start()
    wait("wd")
    start()

    def dbody(j, acc):
        off = pl.multiple_of(j * _STEP, _STEP)
        return acc + lax.dot_general(
            h_s[:, pl.ds(off, _STEP)].astype(_BF), wd[:, pl.ds(off, _STEP)], _NT,
            preferred_element_type=_F32)

    d = lax.fori_loop(0, F // _STEP, dbody, jnp.zeros((8, D), _F32))
    gate = jax.nn.silu(d)
    start(nwo)
    acc = jnp.zeros((8, D), _F32)
    for i in range(nwo):
        wait(f"wo{i}")
        a, b = bounds[i], bounds[i + 1]
        n = (b - a) // _STEP
        if n >= 2:
            def obody(j, acc, a=a):
                off = pl.multiple_of(a + j * _STEP, 128)
                return acc + lax.dot_general(
                    o_s[:, pl.ds(off, _STEP)].astype(_BF), wo[:, pl.ds(off, _STEP)], _NT,
                    preferred_element_type=_F32)

            acc = lax.fori_loop(0, n, obody, acc)
            a += n * _STEP
        if b > a:
            acc = acc + lax.dot_general(
                o_s[:, a:b].astype(_BF), wo[:, a:b], _NT, preferred_element_type=_F32)
    o_ref[...] = (x + (acc * gate)[0:1]).astype(o_ref.dtype)


@jax.jit
def pallas_recurrent_scan__sliding_block_cached__glu_gated_glu__decode_kernel(
    A_x: jax.Array,
    A_k_cache: jax.Array,
    A_v_cache: jax.Array,
    A_wq: jax.Array,
    A_wo: jax.Array,
    B_x: jax.Array,
    B_w_gate: jax.Array,
    B_w_up: jax.Array,
    B_w_down: jax.Array,
):
    del B_x
    B, Sq, D = A_x.shape
    _, HKV, SK, DH = A_k_cache.shape
    F = B_w_gate.shape[1]
    W = min(4096, max(256, SK // 4))
    Q = _HQ * _DH
    assert (B, Sq, DH, 2 * HKV) == (1, 1, _DH, _HQ)
    bounds = [0]
    for n in _WO_SLABS:
        bounds.append(bounds[-1] + 128 * n)
    assert bounds[-1] == Q

    hbm = pl.BlockSpec(memory_space=pl.ANY)
    dt = A_x.dtype
    out = pl.pallas_call(
        functools.partial(_kernel, bounds=tuple(bounds)),
        in_specs=[hbm] * 8,
        out_specs=pl.BlockSpec(memory_space=pltpu.VMEM),
        out_shape=jax.ShapeDtypeStruct((1, D), dt),
        scratch_shapes=[
            pltpu.VMEM((1, D), dt),
            pltpu.VMEM((HKV, W, DH), dt),
            pltpu.VMEM((HKV, W, DH), dt),
            pltpu.VMEM((D, Q), dt),
            pltpu.VMEM((D, Q), dt),
            pltpu.VMEM((D, F), dt),
            pltpu.VMEM((D, F), dt),
            pltpu.VMEM((D, F), dt),
            pltpu.VMEM((HKV, 8, DH), _F32),
            pltpu.VMEM((HKV, 8, W), _F32),
            pltpu.VMEM((HKV, 8, DH), _F32),
            pltpu.VMEM((8, F), _F32),
            pltpu.VMEM((8, F), _F32),
            pltpu.VMEM((8, Q), _F32),
            pltpu.SemaphoreType.DMA((7,)),
            pltpu.SemaphoreType.DMA((len(_WO_SLABS),)),
        ],
        compiler_params=pltpu.CompilerParams(vmem_limit_bytes=100 * 2**20),
    )(A_x.reshape(1, D), A_k_cache, A_v_cache, A_wq, A_wo.T, B_w_gate, B_w_up, B_w_down.T)
    return out.reshape(B, Sq, D)
```

```python
import functools

import jax
import jax.numpy as jnp
from jax import lax
import jax.experimental.pallas as pl
import jax.experimental.pallas.tpu as pltpu

_BF = jnp.bfloat16
_F32 = jnp.float32
_NT = (((1,), (1,)), ((), ()))
_NN = (((1,), (0,)), ((), ()))

_HQ, _DH = 32, 128
_STEP = 512
_OSTEP = 1024


def _kernel(x_hbm, k_hbm, v_hbm, wq_hbm, woT_hbm, wg_hbm, wu_hbm, wdT_hbm, o_ref,
            xb, kb, vb, wq, wo, wg, wu, wd, q_s, p_s, l_s, g_s, h_s, o_s, sems, osem,
            *, bounds):
    D = xb.shape[1]
    HKV, W, DH = kb.shape
    SK = k_hbm.shape[2]
    F = wg.shape[1]
    GRP = 2 * DH
    nwo = len(bounds) - 1

    def cp(src, dst, i):
        return pltpu.make_async_copy(src, dst, sems.at[i])

    def cwo(i):
        a, b = bounds[i], bounds[i + 1]
        return pltpu.make_async_copy(
            woT_hbm.at[pl.ds(a, b - a)], wo.at[pl.ds(a, b - a)], osem.at[i])

    mk = dict(
        x=lambda: cp(x_hbm, xb, 0),
        wq=lambda: cp(wq_hbm, wq, 1),
        k=lambda: cp(k_hbm.at[0, :, pl.ds(SK - W, W), :], kb, 2),
        v=lambda: cp(v_hbm.at[0, :, pl.ds(SK - W, W), :], vb, 3),
        wg=lambda: cp(wg_hbm, wg, 4),
        wu=lambda: cp(wu_hbm, wu, 5),
        wd=lambda: cp(wdT_hbm, wd, 6),
    )
    for i in range(nwo):
        mk[f"wo{i}"] = functools.partial(cwo, i)
    todo = ["x", "wq", "k", "v", "wg", "wu", "wd"] + [f"wo{i}" for i in range(nwo)]

    def start(n=1):
        for _ in range(n):
            if todo:
                mk[todo.pop(0)]().start()

    def wait(name):
        mk[name]().wait()

    start(3)
    wait("x")
    x = xb[...].astype(_F32)
    m = jnp.mean(x, axis=-1, keepdims=True)
    xc = x - m
    var = jnp.mean(xc * xc, axis=-1, keepdims=True)
    xn = xc / jnp.sqrt(var + 1e-5)
    xn8 = jnp.broadcast_to(xn, (8, D)).astype(_BF)
    row = lax.broadcasted_iota(jnp.int32, (8, DH), 0)

    wait("wq")

    def qbody(h, c):
        off = pl.multiple_of(h * GRP, GRP)
        q = lax.dot_general(xn8, wq[:, pl.ds(off, GRP)], _NN, preferred_element_type=_F32)
        q_s[h] = jnp.where(row == 0, q[:, :DH], q[:, DH:])
        return c

    lax.fori_loop(0, HKV, qbody, 0)
    start()
    wait("k")

    def sbody(h, c):
        q = q_s[h].astype(_BF)
        s = lax.dot_general(q, kb[h], _NT, preferred_element_type=_F32) * (DH ** -0.5)
        mx = jnp.max(s, axis=-1, keepdims=True)
        p = jnp.exp(s - mx)
        l_s[h] = jnp.broadcast_to(jnp.sum(p, axis=-1, keepdims=True), (8, DH))
        p_s[h] = p
        return c

    lax.fori_loop(0, HKV, sbody, 0)
    start()
    wait("v")
    start()

    def pvbody(h, c):
        o = lax.dot_general(p_s[h].astype(_BF), vb[h], _NN, preferred_element_type=_F32) / l_s[h]
        off = pl.multiple_of(h * GRP, GRP)
        o_s[:, pl.ds(off, GRP)] = jnp.concatenate(
            [jnp.broadcast_to(o[0:1], (8, DH)), jnp.broadcast_to(o[1:2], (8, DH))], axis=1)
        return c

    lax.fori_loop(0, HKV, pvbody, 0)
    start()
    wait("wg")

    def gbody(j, c):
        off = pl.multiple_of(j * _STEP, _STEP)
        g = lax.dot_general(xn8, wg[:, pl.ds(off, _STEP)], _NN, preferred_element_type=_F32)
        g_s[:, pl.ds(off, _STEP)] = jax.nn.sigmoid(g)
        return c

    lax.fori_loop(0, F // _STEP, gbody, 0)
    start()
    wait("wu")
    start()

    def ubody(j, c):
        off = pl.multiple_of(j * _STEP, _STEP)
        u = lax.dot_general(xn8, wu[:, pl.ds(off, _STEP)], _NN, preferred_element_type=_F32)
        h_s[:, pl.ds(off, _STEP)] = g_s[:, pl.ds(off, _STEP)] * u
        return c

    lax.fori_loop(0, F // _STEP, ubody, 0)
    start()
    wait("wd")
    start()

    def dbody(j, acc):
        off = pl.multiple_of(j * _STEP, _STEP)
        return acc + lax.dot_general(
            h_s[:, pl.ds(off, _STEP)].astype(_BF), wd[:, pl.ds(off, _STEP)], _NT,
            preferred_element_type=_F32)

    d = lax.fori_loop(0, F // _STEP, dbody, jnp.zeros((8, D), _F32))
    gate = jax.nn.silu(d)
    start(nwo)
    for i in range(nwo):
        wait(f"wo{i}")
        a, b = bounds[i], bounds[i + 1]
        if b - a > 128:
            def obody(j, acc, a=a, b=b):
                off = pl.multiple_of(j * _OSTEP, _OSTEP)
                return acc + lax.dot_general(
                    o_s[:, pl.ds(off, _OSTEP)].astype(_BF), wo[a:b, pl.ds(off, _OSTEP)], _NT,
                    preferred_element_type=_F32)

            acc = lax.fori_loop(0, HKV * GRP // _OSTEP, obody, jnp.zeros((8, b - a), _F32))
        else:
            acc = lax.dot_general(
                o_s[...].astype(_BF), wo[a:b, :], _NT, preferred_element_type=_F32)
        o_ref[:, a:b] = (x[:, a:b] + (acc * gate[:, a:b])[0:1]).astype(o_ref.dtype)


@jax.jit
def pallas_recurrent_scan__sliding_block_cached__glu_gated_glu__decode_kernel(
    A_x: jax.Array,
    A_k_cache: jax.Array,
    A_v_cache: jax.Array,
    A_wq: jax.Array,
    A_wo: jax.Array,
    B_x: jax.Array,
    B_w_gate: jax.Array,
    B_w_up: jax.Array,
    B_w_down: jax.Array,
):
    del B_x
    B, Sq, D = A_x.shape
    _, HKV, SK, DH = A_k_cache.shape
    F = B_w_gate.shape[1]
    W = min(4096, max(256, SK // 4))
    Q = _HQ * _DH
    assert (B, Sq, DH, 2 * HKV) == (1, 1, _DH, _HQ)
    assert D % 128 and D > 256 and F % _STEP == 0 and Q % _OSTEP == 0
    last = D // 128 * 128
    bounds = (0, last - 128, last, D)

    hbm = pl.BlockSpec(memory_space=pl.ANY)
    dt = A_x.dtype
    out = pl.pallas_call(
        functools.partial(_kernel, bounds=bounds),
        in_specs=[hbm] * 8,
        out_specs=pl.BlockSpec(memory_space=pltpu.VMEM),
        out_shape=jax.ShapeDtypeStruct((1, D), dt),
        scratch_shapes=[
            pltpu.VMEM((1, D), dt),
            pltpu.VMEM((HKV, W, DH), dt),
            pltpu.VMEM((HKV, W, DH), dt),
            pltpu.VMEM((D, Q), dt),
            pltpu.VMEM((D, Q), dt),
            pltpu.VMEM((D, F), dt),
            pltpu.VMEM((D, F), dt),
            pltpu.VMEM((D, F), dt),
            pltpu.VMEM((HKV, 8, DH), _F32),
            pltpu.VMEM((HKV, 8, W), _F32),
            pltpu.VMEM((HKV, 8, DH), _F32),
            pltpu.VMEM((8, F), _F32),
            pltpu.VMEM((8, F), _F32),
            pltpu.VMEM((8, Q), _F32),
            pltpu.SemaphoreType.DMA((7,)),
            pltpu.SemaphoreType.DMA((len(bounds) - 1,)),
        ],
        compiler_params=pltpu.CompilerParams(vmem_limit_bytes=100 * 2**20),
    )(A_x.reshape(1, D), A_k_cache, A_v_cache, A_wq, A_wo.T, B_w_gate, B_w_up, B_w_down.T)
    return out.reshape(B, Sq, D)
```
